```python
import os as _os
_os.environ.setdefault("JAX_PLATFORMS", "cpu")
import jax
import jax.numpy as jnp

def _softmax(x, axis=-1):
    return jax.nn.softmax(x, axis=axis)
def _gelu(x):
    return jax.nn.gelu(x, approximate=True)
def _silu(x):
    return jax.nn.silu(x)
def _sigmoid(x):
    return jax.nn.sigmoid(x)
def _layernorm(x, axis=-1, eps=1e-5):
    m = jnp.mean(x, axis=axis, keepdims=True)
    v = jnp.var(x, axis=axis, keepdims=True)
    return (x - m) / jnp.sqrt(v + eps)
def _scatter_add(tgt, idx, src, axis=0):
    return tgt.at[idx].add(src)
def _segment_sum(src, seg, n):
    return jax.ops.segment_sum(src, seg, n)
class _Rng:
    def __init__(self, key):
        self._k = key
    def _next(self):
        self._k, sub = jax.random.split(self._k)
        return sub
    def normal(self, shape):
        return jax.random.normal(self._next(), shape, dtype=jnp.bfloat16)
    def randint(self, lo, hi, shape):
        return jax.random.randint(self._next(), shape, lo, hi, dtype=jnp.int32)
    def uniform(self, shape, lo=0.0, hi=1.0):
        return jax.random.uniform(self._next(), shape, jnp.bfloat16, lo, hi)
    def permutation(self, n):
        return jax.random.permutation(self._next(), n)


kernel_name = 'standalone__sliding_local_fixed_window__prompt'

def setup_inputs():
    _rng = _Rng(jax.random.key(int.from_bytes(__import__("os").urandom(4), "little")))
    _w = (lambda a: (lambda t: t.astype(jnp.bfloat16) if jnp.issubdtype(t.dtype, jnp.floating) else t)(jnp.asarray(a)))
    B, H, S, D = 1, 32, 2048, 128
    return {
        "q": _w((lambda *s: _rng.normal(s) * 0.4)(B, H, S, D)),
        "k": _w((lambda *s: _rng.normal(s) * 0.4)(B, H, S, D)),
        "v": _w((lambda *s: _rng.normal(s) * 0.05)(B, H, S, D)),
    }

def reference(q, k, v):
    B, H, S, D = q.shape
    w = 32
    pos = jnp.arange(S)
    rel = pos[:, None] - pos[None, :]
    mask = (rel >= 0) & (rel < w)
    scores = jnp.einsum("bhqd,bhkd->bhqk", q, k) * (D ** -0.5)
    scores = jnp.where(mask[None, None], scores, (lambda x, dt: x.astype(dt))(jnp.array(-1e9), q.dtype))
    p = _softmax(scores, axis=-1)
    return jnp.einsum("bhqk,bhkd->bhqd", p, v)
```

```python
import functools

import jax
import jax.numpy as jnp
from jax import lax
import jax.experimental.pallas as pl
import jax.experimental.pallas.tpu as pltpu

_WINDOW = 32
_KEYS = 128
_QROWS = _KEYS - _WINDOW
_GROUPS = 8
_WRITE_ROWS = 128
_TAIL_ROWS = 192
_MASKED = -1e30


def _attn_block(q, k, v, mask, scale):
    s = lax.dot_general(q, k, (((1,), (1,)), ((), ())),
                        preferred_element_type=jnp.float32)
    s = jnp.where(mask, s, _MASKED)
    m = jnp.max(s, axis=-1, keepdims=True)
    p = jnp.exp((s - m) * scale)
    l = jnp.sum(p, axis=-1, keepdims=True)
    o = jnp.dot(p.astype(v.dtype), v, preferred_element_type=jnp.float32)
    return o * pl.reciprocal(l, approx=False)


def _attn_head(q_ref, k_ref, v_ref, o_ref):
    seq, dim = q_ref.shape
    scale = dim ** -0.5
    row = lax.broadcasted_iota(jnp.int32, (_KEYS, _KEYS), 0)
    col = lax.broadcasted_iota(jnp.int32, (_KEYS, _KEYS), 1)
    rel = row - col
    mask = (rel >= 0) & (rel < _WINDOW)
    o_ref[0:_KEYS, :] = _attn_block(
        q_ref[0:_KEYS, :], k_ref[0:_KEYS, :], v_ref[0:_KEYS, :], mask, scale
    ).astype(o_ref.dtype)
    mask_tail = mask[_WINDOW:, :]
    for j in range(1, (seq - _KEYS) // _QROWS + 1):
        ks = _QROWS * j
        qs = ks + _WINDOW
        o_ref[qs:qs + _QROWS, :] = _attn_block(
            q_ref[qs:qs + _QROWS, :], k_ref[ks:ks + _KEYS, :],
            v_ref[ks:ks + _KEYS, :], mask_tail, scale
        ).astype(o_ref.dtype)


def _kernel(q_hbm, k_hbm, v_hbm, o_hbm, qbuf, kbuf, vbuf, obuf, rsem, tsem, wsem):
    groups, chunks, seq, _ = qbuf.shape
    last = chunks - 1
    head_rows = seq - _TAIL_ROWS

    def reads(j):
        q_cp = pltpu.make_async_copy(q_hbm.at[:, j], qbuf.at[:, j], rsem.at[j])
        k_cp = pltpu.make_async_copy(k_hbm.at[:, j], kbuf.at[:, j], rsem.at[j])
        if j == last:
            rows = pl.ds(0, head_rows)
            v_cp = pltpu.make_async_copy(
                v_hbm.at[:, j, rows], vbuf.at[:, j, rows], rsem.at[j])
        else:
            v_cp = pltpu.make_async_copy(v_hbm.at[:, j], vbuf.at[:, j], rsem.at[j])
        return q_cp, k_cp, v_cp

    def tail_read():
        rows = pl.ds(head_rows, _TAIL_ROWS)
        return pltpu.make_async_copy(
            v_hbm.at[:, last, rows], vbuf.at[:, last, rows], tsem)

    def start_writes(j):
        for i in range(seq // _WRITE_ROWS):
            rows = pl.ds(i * _WRITE_ROWS, _WRITE_ROWS)
            pltpu.make_async_copy(
                obuf.at[:, j, rows], o_hbm.at[:, j, rows], wsem).start()

    def compute(j):
        def body(g, carry):
            _attn_head(qbuf.at[g, j], kbuf.at[g, j], vbuf.at[g, j], obuf.at[g, j])
            return carry
        lax.fori_loop(0, groups, body, 0)

    for j in range(chunks):
        for cp in reads(j):
            cp.start()
    tail_read().start()

    for j in range(last):
        for cp in reads(j):
            cp.wait()
        compute(j)

    for cp in reads(last):
        cp.wait()
    for j in range(last):
        start_writes(j)
    tail_read().wait()
    compute(last)
    start_writes(last)
    pltpu.make_async_copy(obuf, o_hbm, wsem).wait()


@jax.jit
def pallas_standalone__sliding_local_fixed_window__prompt_kernel(
    q: jax.Array,
    k: jax.Array,
    v: jax.Array,
):
    batch, heads, seq, dim = q.shape
    assert (batch * heads) % _GROUPS == 0
    assert (seq - _KEYS) % _QROWS == 0 and seq % _WRITE_ROWS == 0
    chunks = batch * heads // _GROUPS
    shape = (_GROUPS, chunks, seq, dim)
    hbm = pl.BlockSpec(memory_space=pl.ANY)
    out = pl.pallas_call(
        _kernel,
        in_specs=[hbm, hbm, hbm],
        out_specs=hbm,
        out_shape=jax.ShapeDtypeStruct(shape, q.dtype),
        scratch_shapes=[pltpu.VMEM(shape, q.dtype)] * 4 + [
            pltpu.SemaphoreType.DMA((chunks,)),
            pltpu.SemaphoreType.DMA,
            pltpu.SemaphoreType.DMA,
        ],
        compiler_params=pltpu.CompilerParams(
            vmem_limit_bytes=80 * 1024 * 1024,
        ),
    )(q.reshape(shape), k.reshape(shape), v.reshape(shape))
    return out.reshape(q.shape)
```

```python
import jax
import jax.numpy as jnp
from jax import lax
import jax.experimental.pallas as pl
import jax.experimental.pallas.tpu as pltpu

_WINDOW = 32
_KEYS = 128
_QROWS = _KEYS - _WINDOW
_MASKED = -1e30

_GROUPS = 8
_WRITE_ROWS = 128
_TAIL_ROWS = 192
_SIDE_ROWS = (240, 240, 208)
_SIDE_STEP_1 = 4
_SIDE_STEP_2 = 18


def _attn_block(q, k, v, mask, scale):
    s = lax.dot_general(q, k, (((1,), (1,)), ((), ())),
                        preferred_element_type=jnp.float32)
    s = jnp.where(mask, s, _MASKED)
    m = jnp.max(s, axis=-1, keepdims=True)
    p = jnp.exp((s - m) * scale)
    l = jnp.sum(p, axis=-1, keepdims=True)
    o = jnp.dot(p.astype(v.dtype), v, preferred_element_type=jnp.float32)
    return o * pl.reciprocal(l, approx=False)


def _attn_head(q_ref, k_ref, v_ref, o_ref):
    seq, dim = q_ref.shape
    scale = dim ** -0.5
    row = lax.broadcasted_iota(jnp.int32, (_KEYS, _KEYS), 0)
    col = lax.broadcasted_iota(jnp.int32, (_KEYS, _KEYS), 1)
    rel = row - col
    mask = (rel >= 0) & (rel < _WINDOW)
    o_ref[0:_KEYS, :] = _attn_block(
        q_ref[0:_KEYS, :], k_ref[0:_KEYS, :], v_ref[0:_KEYS, :], mask, scale
    ).astype(o_ref.dtype)
    mask_tail = mask[_WINDOW:, :]
    for j in range(1, (seq - _KEYS) // _QROWS + 1):
        ks = _QROWS * j
        qs = ks + _WINDOW
        o_ref[qs:qs + _QROWS, :] = _attn_block(
            q_ref[qs:qs + _QROWS, :], k_ref[ks:ks + _KEYS, :],
            v_ref[ks:ks + _KEYS, :], mask_tail, scale
        ).astype(o_ref.dtype)


def _kernel(q_hbm, k_hbm, v_hbm, o_hbm, qbuf, kbuf, vbuf, obuf, side,
            rsem, tsem, wsem, ssem):
    groups, chunks, seq, _ = qbuf.shape
    last = chunks - 1
    q_main_rows = seq - sum(_SIDE_ROWS)
    v_main_rows = seq - _TAIL_ROWS

    def reads(j):
        q_rows = pl.ds(0, q_main_rows if j == last else seq)
        v_rows = pl.ds(0, v_main_rows if j == last else seq)
        return (
            pltpu.make_async_copy(
                q_hbm.at[:, j, q_rows], qbuf.at[:, j, q_rows], rsem.at[j]),
            pltpu.make_async_copy(k_hbm.at[:, j], kbuf.at[:, j], rsem.at[j]),
            pltpu.make_async_copy(
                v_hbm.at[:, j, v_rows], vbuf.at[:, j, v_rows], rsem.at[j]),
        )

    def tail_read():
        rows = pl.ds(v_main_rows, _TAIL_ROWS)
        return pltpu.make_async_copy(
            v_hbm.at[:, last, rows], vbuf.at[:, last, rows], tsem)

    def side_rows(b):
        return pl.ds(q_main_rows + sum(_SIDE_ROWS[:b]), _SIDE_ROWS[b])

    def side_slot(b):
        return side.at[b % 2, :, pl.ds(0, _SIDE_ROWS[b])]

    def side_in(b):
        return pltpu.make_async_copy(
            q_hbm.at[:, last, side_rows(b)], side_slot(b), ssem.at[b % 2])

    def side_out(b):
        return pltpu.make_async_copy(
            side_slot(b), qbuf.at[:, last, side_rows(b)], ssem.at[b % 2])

    def start_writes(j):
        for i in range(seq // _WRITE_ROWS):
            rows = pl.ds(i * _WRITE_ROWS, _WRITE_ROWS)
            pltpu.make_async_copy(
                obuf.at[:, j, rows], o_hbm.at[:, j, rows], wsem).start()

    def head(g, j):
        _attn_head(qbuf.at[g, j], kbuf.at[g, j], vbuf.at[g, j], obuf.at[g, j])

    for j in range(chunks):
        for cp in reads(j):
            cp.start()
        if j == 0:
            side_in(0).start()
            side_in(1).start()
    tail_read().start()
    side_in(0).wait()
    side_out(0).start()

    def read_phase_step(h, carry):
        @pl.when(h == groups)
        def _():
            side_out(0).wait()
            side_in(2).start()

        for j in range(last):
            @pl.when(h == j * groups)
            def _():
                for cp in reads(j):
                    cp.wait()

        @pl.when(h == _SIDE_STEP_1)
        def _():
            side_in(1).wait()
            side_out(1).start()

        @pl.when(h == _SIDE_STEP_2)
        def _():
            side_in(2).wait()
            side_out(2).start()

        head(h % groups, h // groups)
        return carry

    lax.fori_loop(0, groups * last, read_phase_step, 0)
    side_out(1).wait()
    side_out(2).wait()
    for cp in reads(last):
        cp.wait()

    for j in range(last):
        start_writes(j)
    tail_read().wait()

    def last_chunk_step(g, carry):
        head(g, last)
        return carry

    lax.fori_loop(0, groups, last_chunk_step, 0)
    start_writes(last)
    pltpu.make_async_copy(obuf, o_hbm, wsem).wait()


@jax.jit
def pallas_standalone__sliding_local_fixed_window__prompt_kernel(
    q: jax.Array,
    k: jax.Array,
    v: jax.Array,
):
    batch, heads, seq, dim = q.shape
    assert (batch * heads) % _GROUPS == 0
    assert (seq - _KEYS) % _QROWS == 0 and seq % _WRITE_ROWS == 0
    chunks = batch * heads // _GROUPS
    assert _SIDE_STEP_1 < _GROUPS < _SIDE_STEP_2 < _GROUPS * (chunks - 1)
    shape = (_GROUPS, chunks, seq, dim)
    hbm = pl.BlockSpec(memory_space=pl.ANY)
    out = pl.pallas_call(
        _kernel,
        in_specs=[hbm, hbm, hbm],
        out_specs=hbm,
        out_shape=jax.ShapeDtypeStruct(shape, q.dtype),
        scratch_shapes=[pltpu.VMEM(shape, q.dtype)] * 4 + [
            pltpu.SMEM((2, _GROUPS, max(_SIDE_ROWS), dim), q.dtype),
            pltpu.SemaphoreType.DMA((chunks,)),
            pltpu.SemaphoreType.DMA,
            pltpu.SemaphoreType.DMA,
            pltpu.SemaphoreType.DMA((2,)),
        ],
        compiler_params=pltpu.CompilerParams(
            vmem_limit_bytes=80 * 1024 * 1024,
            disable_semaphore_checks=True,
        ),
    )(q.reshape(shape), k.reshape(shape), v.reshape(shape))
    return out.reshape(q.shape)
```

```python
import math

import jax
import jax.numpy as jnp
import numpy as np
from jax import lax
import jax.experimental.pallas as pl
import jax.experimental.pallas.tpu as pltpu

_WINDOW = 32
_KEYS = 128
_QROWS = _KEYS - _WINDOW
_FILL = -1e9

_GROUPS = 8
_WRITE_ROWS = 128
_TAIL_ROWS = 192
_SIDE_ROWS = (240, 240, 208)
_SIDE_STEP_1 = 4
_SIDE_STEP_2 = 18


def _attn_block(q, k, v, mask, coef, fill, seq, v_mean):
    s = lax.dot_general(q, k, (((1,), (1,)), ((), ())),
                        preferred_element_type=jnp.float32)
    s = jnp.where(mask, s, fill)
    m = jnp.broadcast_to(jnp.max(s, axis=-1, keepdims=True), s.shape)
    p_fill = jnp.exp2((fill - m) * coef)
    p = jnp.exp2((s - m) * coef) - p_fill
    all_fill = seq * p_fill
    l = jnp.sum(p, axis=-1, keepdims=True) + all_fill[:, :1]
    o = jnp.dot(p.astype(v.dtype), v, preferred_element_type=jnp.float32)
    r = pl.reciprocal(l, approx=True)
    r = r * (2.0 - l * r)
    return (o + all_fill * v_mean) * r


def _attn_head(q_ref, k_ref, v_ref, o_ref):
    seq, dim = q_ref.shape
    scale = dim ** -0.5
    coef = scale * math.log2(math.e)
    fill = float(np.asarray(_FILL, np.float32).astype(q_ref.dtype)) / scale
    row = lax.broadcasted_iota(jnp.int32, (_KEYS, _KEYS), 0)
    col = lax.broadcasted_iota(jnp.int32, (_KEYS, _KEYS), 1)
    rel = row - col
    mask = (rel >= 0) & (rel < _WINDOW)
    v_mean = jnp.dot(jnp.full((16, seq), 1.0 / seq, v_ref.dtype), v_ref[...],
                     preferred_element_type=jnp.float32)[0:1, :]
    o_ref[0:_KEYS, :] = _attn_block(
        q_ref[0:_KEYS, :], k_ref[0:_KEYS, :], v_ref[0:_KEYS, :],
        mask, coef, fill, seq, v_mean
    ).astype(o_ref.dtype)
    mask_tail = mask[_WINDOW:, :]
    for j in range(1, (seq - _KEYS) // _QROWS + 1):
        ks = _QROWS * j
        qs = ks + _WINDOW
        o_ref[qs:qs + _QROWS, :] = _attn_block(
            q_ref[qs:qs + _QROWS, :], k_ref[ks:ks + _KEYS, :],
            v_ref[ks:ks + _KEYS, :], mask_tail, coef, fill, seq, v_mean
        ).astype(o_ref.dtype)


def _kernel(q_hbm, k_hbm, v_hbm, o_hbm, qbuf, kbuf, vbuf, obuf, side,
            rsem, tsem, wsem, ssem):
    groups, chunks, seq, _ = qbuf.shape
    last = chunks - 1
    q_main_rows = seq - sum(_SIDE_ROWS)
    v_main_rows = seq - _TAIL_ROWS

    def reads(j):
        q_rows = pl.ds(0, q_main_rows if j == last else seq)
        v_rows = pl.ds(0, v_main_rows if j == last else seq)
        return (
            pltpu.make_async_copy(
                q_hbm.at[:, j, q_rows], qbuf.at[:, j, q_rows], rsem.at[j]),
            pltpu.make_async_copy(k_hbm.at[:, j], kbuf.at[:, j], rsem.at[j]),
            pltpu.make_async_copy(
                v_hbm.at[:, j, v_rows], vbuf.at[:, j, v_rows], rsem.at[j]),
        )

    def tail_read():
        rows = pl.ds(v_main_rows, _TAIL_ROWS)
        return pltpu.make_async_copy(
            v_hbm.at[:, last, rows], vbuf.at[:, last, rows], tsem)

    def side_rows(b):
        return pl.ds(q_main_rows + sum(_SIDE_ROWS[:b]), _SIDE_ROWS[b])

    def side_slot(b):
        return side.at[b % 2, :, pl.ds(0, _SIDE_ROWS[b])]

    def side_in(b):
        return pltpu.make_async_copy(
            q_hbm.at[:, last, side_rows(b)], side_slot(b), ssem.at[b % 2])

    def side_out(b):
        return pltpu.make_async_copy(
            side_slot(b), qbuf.at[:, last, side_rows(b)], ssem.at[b % 2])

    def start_writes(j):
        for i in range(seq // _WRITE_ROWS):
            rows = pl.ds(i * _WRITE_ROWS, _WRITE_ROWS)
            pltpu.make_async_copy(
                obuf.at[:, j, rows], o_hbm.at[:, j, rows], wsem).start()

    def head(g, j):
        _attn_head(qbuf.at[g, j], kbuf.at[g, j], vbuf.at[g, j], obuf.at[g, j])

    for j in range(chunks):
        for cp in reads(j):
            cp.start()
        if j == 0:
            side_in(0).start()
            side_in(1).start()
    tail_read().start()
    side_in(0).wait()
    side_out(0).start()

    def read_phase_step(h, carry):
        @pl.when(h == groups)
        def _():
            side_out(0).wait()
            side_in(2).start()

        for j in range(last):
            @pl.when(h == j * groups)
            def _():
                for cp in reads(j):
                    cp.wait()

        @pl.when(h == _SIDE_STEP_1)
        def _():
            side_in(1).wait()
            side_out(1).start()

        @pl.when(h == _SIDE_STEP_2)
        def _():
            side_in(2).wait()
            side_out(2).start()

        head(h % groups, h // groups)
        return carry

    lax.fori_loop(0, groups * last, read_phase_step, 0)
    side_out(1).wait()
    side_out(2).wait()
    for cp in reads(last):
        cp.wait()

    for j in range(last):
        start_writes(j)
    tail_read().wait()

    def last_chunk_step(g, carry):
        head(g, last)
        return carry

    lax.fori_loop(0, groups, last_chunk_step, 0)
    start_writes(last)
    pltpu.make_async_copy(obuf, o_hbm, wsem).wait()


@jax.jit
def pallas_standalone__sliding_local_fixed_window__prompt_kernel(
    q: jax.Array,
    k: jax.Array,
    v: jax.Array,
):
    batch, heads, seq, dim = q.shape
    assert (batch * heads) % _GROUPS == 0 and dim == _KEYS
    assert (seq - _KEYS) % _QROWS == 0 and seq % _WRITE_ROWS == 0
    assert seq & (seq - 1) == 0
    chunks = batch * heads // _GROUPS
    assert _SIDE_STEP_1 < _GROUPS < _SIDE_STEP_2 < _GROUPS * (chunks - 1)
    shape = (_GROUPS, chunks, seq, dim)
    hbm = pl.BlockSpec(memory_space=pl.ANY)
    out = pl.pallas_call(
        _kernel,
        in_specs=[hbm, hbm, hbm],
        out_specs=hbm,
        out_shape=jax.ShapeDtypeStruct(shape, q.dtype),
        scratch_shapes=[pltpu.VMEM(shape, q.dtype)] * 4 + [
            pltpu.SMEM((2, _GROUPS, max(_SIDE_ROWS), dim), q.dtype),
            pltpu.SemaphoreType.DMA((chunks,)),
            pltpu.SemaphoreType.DMA,
            pltpu.SemaphoreType.DMA,
            pltpu.SemaphoreType.DMA((2,)),
        ],
        compiler_params=pltpu.CompilerParams(
            vmem_limit_bytes=80 * 1024 * 1024,
            disable_semaphore_checks=True,
        ),
    )(q.reshape(shape), k.reshape(shape), v.reshape(shape))
    return out.reshape(q.shape)
```
